```python
import jax
import jax.numpy as jnp

def _softmax(x, axis=-1):
    return jax.nn.softmax(x, axis=axis)
def _gelu(x):
    return jax.nn.gelu(x, approximate=True)
def _silu(x):
    return jax.nn.silu(x)
def _sigmoid(x):
    return jax.nn.sigmoid(x)
def _layernorm(x, axis=-1, eps=1e-5):
    m = jnp.mean(x, axis=axis, keepdims=True)
    v = jnp.var(x, axis=axis, keepdims=True)
    return (x - m) / jnp.sqrt(v + eps)
def _scatter_add(tgt, idx, src, axis=0):
    return tgt.at[idx].add(src)
def _segment_sum(src, seg, n):
    return jax.ops.segment_sum(src, seg, n)
class _Rng:
    def __init__(self, key):
        self._k = key
    def _next(self):
        self._k, sub = jax.random.split(self._k)
        return sub
    def normal(self, shape):
        return jax.random.normal(self._next(), shape, dtype=jnp.bfloat16)
    def randint(self, lo, hi, shape):
        return jax.random.randint(self._next(), shape, lo, hi, dtype=jnp.int32)
    def uniform(self, shape, lo=0.0, hi=1.0):
        return jax.random.uniform(self._next(), shape, jnp.bfloat16, lo, hi)
    def permutation(self, n):
        return jax.random.permutation(self._next(), n)


kernel_name = 'sequential_preLN__grouped_kv_mqa__glu_gated_swiglu__prompt'

def _fwd_setup_inputs():
    _rng = _Rng(jax.random.key(int.from_bytes(__import__("os").urandom(4), "little")))
    _w = (lambda a: (lambda t: t.astype(jnp.bfloat16) if jnp.issubdtype(t.dtype, jnp.floating) else t)(jnp.asarray(a)))
    def _A_setup():
        B, S, D, H = 1, 2048, 512, 32
        Dh = D // H
        return {
            "x": _w((lambda *s: _rng.normal(s) * 0.05)(B, S, D)),
            "wq": _w((lambda *s: _rng.normal(s) * 0.05)(D, H * Dh)),
            "wk": _w((lambda *s: _rng.normal(s) * 0.05)(D, Dh)),
            "wv": _w((lambda *s: _rng.normal(s) * 0.05)(D, Dh)),
            "wo": _w((lambda *s: _rng.normal(s) * 0.05)(H * Dh, D)),
        }
    _A_in = _A_setup()

    def _B_setup():
        B, S, D, F = 1, 2048, 512, 1376
        return {
            "x": _w((lambda *s: _rng.normal(s) * 0.05)(B, S, D)),
            "w1": _w((lambda *s: _rng.normal(s) * 0.05)(D, F) * (2.0 / D) ** 0.5),
            "w3": _w((lambda *s: _rng.normal(s) * 0.05)(D, F) * (2.0 / D) ** 0.5),
            "w2": _w((lambda *s: _rng.normal(s) * 0.05)(F, D) * (2.0 / F) ** 0.5),
        }
    _B_in = _B_setup()

    return {
        "A_x": _A_in["x"],
        "A_wq": _A_in["wq"],
        "A_wk": _A_in["wk"],
        "A_wv": _A_in["wv"],
        "A_wo": _A_in["wo"],
        "B_x": _B_in["x"],
        "B_w1": _B_in["w1"],
        "B_w3": _B_in["w3"],
        "B_w2": _B_in["w2"],
    }

def _fwd_reference(A_x, A_wq, A_wk, A_wv, A_wo, B_x, B_w1, B_w3, B_w2):
    def _A_ref(x, wq, wk, wv, wo):
        B, S, D = x.shape
        H = 32
        Dh = D // H
        q = (lambda x, *d: x.transpose(*d))((x @ wq).reshape(B, S, H, Dh), 0, 2, 1, 3)
        k = x @ wk
        v = x @ wv
        scores = jnp.einsum("bhqd,bkd->bhqk", q, k) * (Dh ** -0.5)
        p = _softmax(scores, axis=-1)
        o = jnp.einsum("bhqk,bkd->bhqd", p, v)
        return (lambda x, *d: x.transpose(*d))(o, 0, 2, 1, 3).reshape(B, S, H * Dh) @ wo

    def _B_ref(x, w1, w3, w2):
        gate = jnp.einsum("bsd,df->bsf", x, w1)
        up = jnp.einsum("bsd,df->bsf", x, w3)
        h = _silu(gate) * up
        out = jnp.einsum("bsf,fd->bsd", h, w2)
        return out

    x = A_x
    h = x + _A_ref(_layernorm(x, axis=-1), A_wq, A_wk, A_wv, A_wo)
    h2 = h + _B_ref(_layernorm(h, axis=-1), B_w1, B_w3, B_w2)
    return h2


def setup_inputs():
    _inp = _fwd_setup_inputs()
    _gk = jax.random.fold_in(jax.random.key(int.from_bytes(__import__("os").urandom(4), "little")), 2**31 - 1)
    _shapes = [[1, 2048, 512]]
    _dtypes = ['bfloat16']
    _gks = jax.random.split(_gk, len(_shapes))
    _gs = [jax.random.normal(k, s, dtype=jnp.dtype(d)) * 0.05 for k, s, d in zip(_gks, _shapes, _dtypes)]
    _inp["grad_out"] = _gs[0]
    return _inp

def reference(A_x, A_wq, A_wk, A_wv, A_wo, B_w1, B_w3, B_w2, B_x, grad_out):
    _const = dict(B_x=B_x)
    def _f(*_d):
        return _fwd_reference(**{'A_x': _d[0], 'A_wq': _d[1], 'A_wk': _d[2], 'A_wv': _d[3], 'A_wo': _d[4], 'B_w1': _d[5], 'B_w3': _d[6], 'B_w2': _d[7], **_const})
    _out, _vjp = jax.vjp(_f, A_x, A_wq, A_wk, A_wv, A_wo, B_w1, B_w3, B_w2)
    _grads = _vjp(grad_out)
    _out0 = jnp.asarray(_out)
    return (_out0, *[jnp.asarray(_g) for _g in _grads])
```

```python
import jax
import jax.numpy as jnp
from jax import lax
from jax.experimental import pallas as pl
from jax.experimental.pallas import tpu as pltpu

_S = 2048
_D = 512
_H = 32
_DH = 16
_F = 1376
_BQ = 256
_NB = _S // _BQ
_NCOL = _H * _BQ
_C = 512
_T = 256
_U = _NCOL // _C
_J = _S // _T

_EPS = 1e-5
_LOG2E = 1.4426950408889634
_LN2 = 0.6931471805599453
_SC = 0.25
_C2 = _SC * _LOG2E

_f32 = jnp.float32
_bf16 = jnp.bfloat16

_NN = (((1,), (0,)), ((), ()))
_NT = (((1,), (1,)), ((), ()))
_TN = (((0,), (0,)), ((), ()))
_T01 = (((0,), (1,)), ((), ()))


def _mm(a, b, dims):
    return lax.dot_general(a, b, dims, preferred_element_type=_f32)


def _ln_fwd(xf):
    m = jnp.mean(xf, axis=-1, keepdims=True)
    xc = xf - m
    v = jnp.mean(xc * xc, axis=-1, keepdims=True)
    rstd = lax.rsqrt(v + _EPS)
    return xc * rstd, rstd


def _ln_bwd(dy, xhat, rstd):
    return rstd * (dy - jnp.mean(dy, axis=-1, keepdims=True)
                   - xhat * jnp.mean(dy * xhat, axis=-1, keepdims=True))


def _attn_fwd(k_ref, qf_ref, v1T_ref, oTf_ref, pT_ref, sa_ref, sb_ref):
    def pass1_chunk(u, j, s_ref, mrun):
        q = qf_ref[:, pl.ds(pl.multiple_of(u * _C, _C), _C)]
        s = jnp.dot(k_ref[j * _T:(j + 1) * _T, :], q, preferred_element_type=_f32)
        s_ref[j * _T:(j + 1) * _T, :] = s
        return jnp.maximum(mrun, s.reshape(_T // 8, 8, _C).max(axis=0))

    def pass2_chunk(u, j, s_ref, m, oacc):
        s = s_ref[j * _T:(j + 1) * _T, :]
        p = jnp.exp2(s - m).astype(_bf16)
        pT_ref[j * _T:(j + 1) * _T, pl.ds(pl.multiple_of(u * _C, _C), _C)] = p
        return oacc + jnp.dot(v1T_ref[:, j * _T:(j + 1) * _T], p, preferred_element_type=_f32)

    neg = jnp.full((8, _C), -jnp.inf, _f32)

    def step(u, m_cur, cur_ref, nxt_ref):
        mr = neg
        oacc = jnp.zeros((32, _C), _f32)
        for j in range(_J):
            mr = pass1_chunk(u + 1, j, nxt_ref, mr)
            oacc = pass2_chunk(u, j, cur_ref, m_cur, oacc)
        oTf_ref[:, pl.ds(pl.multiple_of(u * _C, _C), _C)] = oacc
        return jnp.max(mr, axis=0, keepdims=True)

    mrun = neg
    for j in range(_J):
        mrun = pass1_chunk(0, j, sa_ref, mrun)
    m0 = jnp.max(mrun, axis=0, keepdims=True)

    def body(p, m_cur):
        m1 = step(2 * p, m_cur, sa_ref, sb_ref)
        return step(2 * p + 1, m1, sb_ref, sa_ref)

    m = lax.fori_loop(0, _U // 2 - 1, body, m0)
    m_last = step(_U - 2, m, sa_ref, sb_ref)
    oacc = jnp.zeros((32, _C), _f32)
    for j in range(_J):
        oacc = pass2_chunk(_U - 1, j, sb_ref, m_last, oacc)
    oTf_ref[:, (_U - 1) * _C:_U * _C] = oacc


def _attn_bwd(v_ref, dof_ref, df_ref, kT_ref, qf_ref, pT_ref, dqf_ref, dkT_ref, dvT_ref):
    def body(u, c):
        cols = pl.ds(pl.multiple_of(u * _C, _C), _C)
        dof = dof_ref[:, cols]
        qf = qf_ref[:, cols]
        d = df_ref[:, cols]

        def dp(j):
            return jnp.dot(v_ref[j * _T:(j + 1) * _T, :], dof, preferred_element_type=_f32)

        def rest(j, dpj, dqacc):
            p = pT_ref[j * _T:(j + 1) * _T, cols]
            ds = (p.astype(_f32) * (dpj - d)).astype(_bf16)
            dqacc = dqacc + jnp.dot(kT_ref[:, j * _T:(j + 1) * _T], ds, preferred_element_type=_f32)
            dkT_ref[:, j * _T:(j + 1) * _T] += _mm(qf, ds, _NT)
            dvT_ref[:, j * _T:(j + 1) * _T] += _mm(dof, p, _NT)
            return dqacc

        dqacc = jnp.zeros((_DH, _C), _f32)
        cur = dp(0)
        for j in range(_J):
            nxt = dp(j + 1) if j + 1 < _J else None
            dqacc = rest(j, cur, dqacc)
            cur = nxt
        dqf_ref[:, cols] = dqacc
        return c

    lax.fori_loop(0, _U, body, 0)


def _kernel(x_ref, wq_ref, wk_ref, wv_ref, wo_ref, w1_ref, w3_ref, w2_ref, g_ref,
            out_ref, dx_ref, dwq_ref, dwk_ref, dwv_ref, dwo_ref, dw1_ref, dw3_ref, dw2_ref,
            ln1_ref, k_ref, v_ref, kT_ref, v1T_ref, qf_ref, dof_ref, df_ref, oTf_ref,
            pT_ref, sa_ref, sb_ref, dqf_ref, oTc_ref, dqTc_ref, dkT_ref, dvT_ref,
            dwq_acc, dwo_acc, dw1_acc, dw3_acc, dw2_acc, dx_acc):
    i = pl.program_id(0)

    @pl.when(i == 0)
    def _prologue():
        def ln_chunk(c, carry):
            r = pl.ds(pl.multiple_of(c * _BQ, _BQ), _BQ)
            xhat, _ = _ln_fwd(x_ref[r, :].astype(_f32))
            ln1_ref[r, :] = xhat.astype(_bf16)
            return carry

        lax.fori_loop(0, _NB, ln_chunk, 0)
        ln1 = ln1_ref[...]
        k_ref[...] = jnp.dot(ln1, wk_ref[...], preferred_element_type=_f32).astype(_bf16)
        v_ref[...] = jnp.dot(ln1, wv_ref[...], preferred_element_type=_f32).astype(_bf16)
        kT_ref[...] = _mm(wk_ref[...], ln1, _T01).astype(_bf16)
        v1T_ref[0:_DH, :] = _mm(wv_ref[...], ln1, _T01).astype(_bf16)
        row = lax.broadcasted_iota(jnp.int32, (_DH, _S), 0)
        v1T_ref[_DH:2 * _DH, :] = jnp.where(row == 0, 1.0, 0.0).astype(_bf16)
        dkT_ref[...] = jnp.zeros_like(dkT_ref)
        dvT_ref[...] = jnp.zeros_like(dvT_ref)
        dwq_acc[...] = jnp.zeros_like(dwq_acc)
        dwo_acc[...] = jnp.zeros_like(dwo_acc)
        dw1_acc[...] = jnp.zeros_like(dw1_acc)
        dw3_acc[...] = jnp.zeros_like(dw3_acc)
        dw2_acc[...] = jnp.zeros_like(dw2_acc)

    rows = pl.ds(pl.multiple_of(i * _BQ, _BQ), _BQ)
    ln1_r = ln1_ref[rows, :]
    xf = x_ref[rows, :].astype(_f32)

    qT = (_mm(wq_ref[...], ln1_r, _T01) * _C2).astype(_bf16)
    for h in range(_H):
        qf_ref[:, h * _BQ:(h + 1) * _BQ] = qT[h * _DH:(h + 1) * _DH, :]

    _attn_fwd(k_ref, qf_ref, v1T_ref, oTf_ref, pT_ref, sa_ref, sb_ref)

    linv = 1.0 / oTf_ref[_DH:_DH + 1, :]
    on = oTf_ref[0:_DH, :] * linv
    for h in range(_H):
        oTc_ref[h * _DH:(h + 1) * _DH, :] = on[:, h * _BQ:(h + 1) * _BQ]
    oTc = oTc_ref[...]
    oTc_b = oTc.astype(_bf16)

    hres = xf + _mm(oTc_b, wo_ref[...], _TN)
    xhat2, rstd2 = _ln_fwd(hres)
    ln2 = xhat2.astype(_bf16)
    gate = jnp.dot(ln2, w1_ref[...], preferred_element_type=_f32)
    up = jnp.dot(ln2, w3_ref[...], preferred_element_type=_f32)
    sig = jax.nn.sigmoid(gate)
    silu = gate * sig
    hh = (silu * up).astype(_bf16)
    out_ref[rows, :] = (hres + jnp.dot(hh, w2_ref[...], preferred_element_type=_f32)).astype(_bf16)

    gb = g_ref[rows, :]
    d_hh = _mm(gb, w2_ref[...], _NT)
    dw2_acc[...] += _mm(hh, gb, _TN)
    d_up = (d_hh * silu).astype(_bf16)
    d_gate = (d_hh * up * (sig * (1.0 + gate * (1.0 - sig)))).astype(_bf16)
    dw1_acc[...] += _mm(ln2, d_gate, _TN)
    dw3_acc[...] += _mm(ln2, d_up, _TN)
    d_ln2 = _mm(d_gate, w1_ref[...], _NT) + _mm(d_up, w3_ref[...], _NT)
    dh = gb.astype(_f32) + _ln_bwd(d_ln2, xhat2, rstd2)
    dhb = dh.astype(_bf16)

    dOT = _mm(wo_ref[...], dhb, _NT)
    dwo_acc[...] += jnp.dot(oTc_b, dhb, preferred_element_type=_f32)
    for h in range(_H):
        li = linv[:, h * _BQ:(h + 1) * _BQ]
        dos = (dOT[h * _DH:(h + 1) * _DH, :] * li).astype(_bf16)
        dof_ref[:, h * _BQ:(h + 1) * _BQ] = dos
        df_ref[:, h * _BQ:(h + 1) * _BQ] = jnp.sum(
            dos.astype(_f32) * oTc[h * _DH:(h + 1) * _DH, :], axis=0, keepdims=True)

    _attn_bwd(v_ref, dof_ref, df_ref, kT_ref, qf_ref, pT_ref, dqf_ref, dkT_ref, dvT_ref)

    dqf = dqf_ref[...] * _SC
    for h in range(_H):
        dqTc_ref[h * _DH:(h + 1) * _DH, :] = dqf[:, h * _BQ:(h + 1) * _BQ]
    dqT_b = dqTc_ref[...].astype(_bf16)
    d_ln1 = _mm(dqT_b, wq_ref[...], _T01)
    dwq_acc[...] += _mm(ln1_r, dqT_b, _T01)
    xhat1, rstd1 = _ln_fwd(xf)
    dx_acc[rows, :] = dh + _ln_bwd(d_ln1, xhat1, rstd1)

    @pl.when(i == _NB - 1)
    def _epilogue():
        dkT_ref[...] = dkT_ref[...] * _LN2
        dkT_b = dkT_ref[...].astype(_bf16)
        dvT_b = dvT_ref[...].astype(_bf16)
        ln1 = ln1_ref[...]
        dwk_ref[...] = _mm(ln1, dkT_b, _T01).astype(_bf16)
        dwv_ref[...] = _mm(ln1, dvT_b, _T01).astype(_bf16)

        def fin(c, carry):
            r = pl.ds(pl.multiple_of(c * _BQ, _BQ), _BQ)
            dl = (_mm(dkT_ref[:, r].astype(_bf16), wk_ref[...], _T01)
                  + _mm(dvT_ref[:, r].astype(_bf16), wv_ref[...], _T01))
            xh, rs = _ln_fwd(x_ref[r, :].astype(_f32))
            dx_ref[r, :] = (dx_acc[r, :] + _ln_bwd(dl, xh, rs)).astype(_bf16)
            return carry

        lax.fori_loop(0, _NB, fin, 0)
        dwq_ref[...] = dwq_acc[...].astype(_bf16)
        dwo_ref[...] = dwo_acc[...].astype(_bf16)
        dw1_ref[...] = dw1_acc[...].astype(_bf16)
        dw3_ref[...] = dw3_acc[...].astype(_bf16)
        dw2_ref[...] = dw2_acc[...].astype(_bf16)


def _full(shape):
    return pl.BlockSpec(shape, lambda i: (0,) * len(shape))


@jax.jit
def pallas_sequential_preLN__grouped_kv_mqa__glu_gated_swiglu__prompt_kernel(
    A_x: jax.Array,
    A_wq: jax.Array,
    A_wk: jax.Array,
    A_wv: jax.Array,
    A_wo: jax.Array,
    B_x: jax.Array,
    B_w1: jax.Array,
    B_w3: jax.Array,
    B_w2: jax.Array,
    grad_out: jax.Array,
):
    del B_x
    x = A_x.reshape(_S, _D)
    g = grad_out.reshape(_S, _D)
    ins = (x, A_wq, A_wk, A_wv, A_wo, B_w1, B_w3, B_w2, g)
    out_shapes = (
        jax.ShapeDtypeStruct((_S, _D), _bf16),
        jax.ShapeDtypeStruct((_S, _D), _bf16),
        jax.ShapeDtypeStruct((_D, _D), _bf16),
        jax.ShapeDtypeStruct((_D, _DH), _bf16),
        jax.ShapeDtypeStruct((_D, _DH), _bf16),
        jax.ShapeDtypeStruct((_D, _D), _bf16),
        jax.ShapeDtypeStruct((_D, _F), _bf16),
        jax.ShapeDtypeStruct((_D, _F), _bf16),
        jax.ShapeDtypeStruct((_F, _D), _bf16),
    )
    scratch = [
        pltpu.VMEM((_S, _D), _bf16),
        pltpu.VMEM((_S, _DH), _bf16),
        pltpu.VMEM((_S, _DH), _bf16),
        pltpu.VMEM((_DH, _S), _bf16),
        pltpu.VMEM((2 * _DH, _S), _bf16),
        pltpu.VMEM((_DH, _NCOL), _bf16),
        pltpu.VMEM((_DH, _NCOL), _bf16),
        pltpu.VMEM((1, _NCOL), _f32),
        pltpu.VMEM((2 * _DH, _NCOL), _f32),
        pltpu.VMEM((_S, _NCOL), _bf16),
        pltpu.VMEM((_S, _C), _f32),
        pltpu.VMEM((_S, _C), _f32),
        pltpu.VMEM((_DH, _NCOL), _f32),
        pltpu.VMEM((_D, _BQ), _f32),
        pltpu.VMEM((_D, _BQ), _f32),
        pltpu.VMEM((_DH, _S), _f32),
        pltpu.VMEM((_DH, _S), _f32),
        pltpu.VMEM((_D, _D), _f32),
        pltpu.VMEM((_D, _D), _f32),
        pltpu.VMEM((_D, _F), _f32),
        pltpu.VMEM((_D, _F), _f32),
        pltpu.VMEM((_F, _D), _f32),
        pltpu.VMEM((_S, _D), _f32),
    ]
    outs = pl.pallas_call(
        _kernel,
        grid=(_NB,),
        in_specs=[_full(a.shape) for a in ins],
        out_specs=[_full(s.shape) for s in out_shapes],
        out_shape=out_shapes,
        scratch_shapes=scratch,
        compiler_params=pltpu.CompilerParams(
            dimension_semantics=("arbitrary",),
            vmem_limit_bytes=120 * 1024 * 1024,
        ),
    )(*ins)
    out, dx = outs[0].reshape(1, _S, _D), outs[1].reshape(1, _S, _D)
    return (out, dx) + tuple(outs[2:])
```

```python
import jax
import jax.numpy as jnp
from jax import lax
from jax.experimental import pallas as pl
from jax.experimental.pallas import tpu as pltpu

_S = 2048
_D = 512
_H = 32
_DH = 16
_F = 1376
_BQ = 256
_NB = _S // _BQ
_NCOL = _H * _BQ
_C = 512
_T = 256
_TB = 128
_U = _NCOL // _C
_J = _S // _T
_JB = _S // _TB
_LAG = 2
_UNR = 4
_TF = 128
_JF = _S // _TF
_LAGF = 2
_UNRF = 4
_THR = 2.0 ** -60
_RB = 128
_NSB = _BQ // _RB

_EPS = 1e-5
_LOG2E = 1.4426950408889634
_LN2 = 0.6931471805599453
_SC = 0.25
_C2 = _SC * _LOG2E

_f32 = jnp.float32
_bf16 = jnp.bfloat16

_NN = (((1,), (0,)), ((), ()))
_NT = (((1,), (1,)), ((), ()))
_TN = (((0,), (0,)), ((), ()))
_T01 = (((0,), (1,)), ((), ()))


def _mm(a, b, dims):
    return lax.dot_general(a, b, dims, preferred_element_type=_f32)


def _ln_fwd(xf):
    m = jnp.mean(xf, axis=-1, keepdims=True)
    xc = xf - m
    v = jnp.mean(xc * xc, axis=-1, keepdims=True)
    rstd = lax.rsqrt(v + _EPS)
    return xc * rstd, rstd


def _ln_bwd(dy, xhat, rstd):
    return rstd * (dy - jnp.mean(dy, axis=-1, keepdims=True)
                   - xhat * jnp.mean(dy * xhat, axis=-1, keepdims=True))


def _pass1_chunk(k_ref, qf_ref, qcol, j, s_ref, mrun):
    q = qf_ref[:, pl.ds(qcol, _C)]
    s = jnp.dot(k_ref[j * _T:(j + 1) * _T, :], q, preferred_element_type=_f32)
    s_ref[j * _T:(j + 1) * _T, :] = s
    return jnp.maximum(mrun, s.reshape(_T // 8, 8, _C).max(axis=0))


def _attn_fwd(k_ref, qf_ref, qbase, v1T_ref, oTf_ref, pT_ref, sa_ref, sb_ref):
    def pass2_chunk(u, j, s_ref, m, oacc):
        s = s_ref[j * _T:(j + 1) * _T, :]
        p = jnp.exp2(s - m).astype(_bf16)
        pT_ref[j * _T:(j + 1) * _T, pl.ds(pl.multiple_of(u * _C, _C), _C)] = p
        r = jnp.dot(v1T_ref[:, j * _T:(j + 1) * _T], p, preferred_element_type=_f32)
        return r if oacc is None else oacc + r

    neg = jnp.full((8, _C), -jnp.inf, _f32)

    def step(u, m_cur, cur_ref, nxt_ref):
        qcol = pl.multiple_of(qbase + (u + 1) * _C, _C)
        mr = neg
        oacc = None
        for j in range(_J):
            mr = _pass1_chunk(k_ref, qf_ref, qcol, j, nxt_ref, mr)
            oacc = pass2_chunk(u, j, cur_ref, m_cur, oacc)
        oTf_ref[:, pl.ds(pl.multiple_of(u * _C, _C), _C)] = oacc
        return jnp.max(mr, axis=0, keepdims=True)

    def body(p, m_cur):
        m1 = step(2 * p, m_cur, sa_ref, sb_ref)
        return step(2 * p + 1, m1, sb_ref, sa_ref)

    mrun = neg
    for j in range(_J):
        mrun = _pass1_chunk(k_ref, qf_ref, pl.multiple_of(qbase, _C), j, sa_ref, mrun)
    m0 = jnp.max(mrun, axis=0, keepdims=True)
    m = lax.fori_loop(0, _U // 2 - 1, body, m0)
    m_last = step(_U - 2, m, sa_ref, sb_ref)
    oacc = None
    for j in range(_J):
        oacc = pass2_chunk(_U - 1, j, sb_ref, m_last, oacc)
    oTf_ref[:, (_U - 1) * _C:_U * _C] = oacc


def _attn_fwd_fast(k_ref, qf_ref, qbase, bq_ref, v1T_ref, oTf_ref, pT_ref):
    def body(pu, c):
        def cols_of(w):
            return pl.ds(pl.multiple_of((pu * _UNRF + w) * _C, _C), _C)

        def qcols_of(w):
            return pl.ds(pl.multiple_of(qbase + (pu * _UNRF + w) * _C, _C), _C)

        def smm(g):
            w, j = divmod(g, _JF)
            return jnp.dot(k_ref[j * _TF:(j + 1) * _TF, :], qf_ref[:, qcols_of(w)],
                           preferred_element_type=_f32)

        acc = {}
        lac = {}
        pend = []

        def pv(g, p):
            w, j = divmod(g, _JF)
            r = jnp.dot(v1T_ref[0:_DH, j * _TF:(j + 1) * _TF], p, preferred_element_type=_f32)
            acc[w] = r if j == 0 else acc[w] + r
            if j == _JF - 1:
                oTf_ref[0:_DH, cols_of(w)] = acc[w]
                oTf_ref[_DH:_DH + 1, cols_of(w)] = jnp.sum(lac[w], axis=0, keepdims=True)

        n = _JF * _UNRF
        s_next = smm(0)
        for g in range(n):
            w, j = divmod(g, _JF)
            sc = s_next
            if g + 1 < n:
                s_next = smm(g + 1)
            pf = jnp.exp2(sc - bq_ref[:, qcols_of(w)])
            ls = pf.reshape(_TF // 8, 8, _C).sum(axis=0)
            lac[w] = ls if j == 0 else lac[w] + ls
            pb = pf.astype(_bf16)
            pT_ref[j * _TF:(j + 1) * _TF, cols_of(w)] = pb
            pend.append((g, pb))
            if len(pend) > _LAGF:
                pv(*pend.pop(0))
        while pend:
            pv(*pend.pop(0))
        return c

    lax.fori_loop(0, _U // _UNRF, body, 0)


def _attn_bwd(v_ref, dof_ref, df_ref, kT_ref, qf_ref, qbase, pT_ref, dqf_ref, dkT_ref, dvT_ref, ds_buf):
    ns = _LAG + 1

    def body(pu, c):
        def cols_of(w):
            return pl.ds(pl.multiple_of((pu * _UNR + w) * _C, _C), _C)

        def qcols_of(w):
            return pl.ds(pl.multiple_of(qbase + (pu * _UNR + w) * _C, _C), _C)

        def pchunk(g):
            w, j = divmod(g, _JB)
            cols = cols_of(w)
            dpj = jnp.dot(v_ref[j * _TB:(j + 1) * _TB, :], dof_ref[:, cols], preferred_element_type=_f32)
            p = pT_ref[j * _TB:(j + 1) * _TB, cols]
            ds_buf[g % ns] = (p.astype(_f32) * (dpj - df_ref[:, cols])).astype(_bf16)

        dq = {}

        def stat(g):
            w, j = divmod(g, _JB)
            cols = cols_of(w)
            rows = slice(j * _TB, (j + 1) * _TB)
            dvT_ref[:, rows] += _mm(dof_ref[:, cols], pT_ref[rows, cols], _NT)
            dkT_ref[:, rows] += _mm(qf_ref[:, qcols_of(w)], ds_buf[g % ns], _NT)
            r = jnp.dot(kT_ref[:, rows], ds_buf[g % ns], preferred_element_type=_f32)
            dq[w] = r if j == 0 else dq[w] + r
            if j == _JB - 1:
                dqf_ref[:, cols] = dq[w]

        n = _JB * _UNR
        for g in range(n + _LAG):
            if g < n:
                pchunk(g)
            if g >= _LAG:
                stat(g - _LAG)
        return c

    lax.fori_loop(0, _U // _UNR, body, 0)


def _qproj(wq_ref, ln1_ref, qf_ref, bq_ref, kmax_ref, blk, qbase):
    rows = pl.ds(pl.multiple_of(blk * _BQ, _BQ), _BQ)
    qT = (_mm(wq_ref[...], ln1_ref[rows, :], _T01) * _C2).astype(_bf16)
    qf32 = qT.astype(_f32)
    bnd = jnp.sqrt((qf32 * qf32).reshape(_H, _DH, _BQ).sum(axis=1)) * kmax_ref[...]
    for h in range(_H):
        lanes = pl.ds(pl.multiple_of(qbase + h * _BQ, _BQ), _BQ)
        qf_ref[:, lanes] = qT[h * _DH:(h + 1) * _DH, :]
        bq_ref[:, lanes] = bnd[h:h + 1, :]


def _kernel(x_hbm, wq_hbm, wkT_hbm, wvT_hbm, wo_hbm, w1T_hbm, w3T_hbm, w2_hbm, g_hbm,
            out_hbm, dx_hbm, dwq_hbm, dwkT_hbm, dwvT_hbm, dwo_hbm, dw1T_hbm, dw3T_hbm, dw2_hbm,
            x_ref, wq_ref, wkT_ref, wvT_ref, wo_ref, w1T_ref, w3T_ref, w2_ref, g_ref,
            out_ref, dx_ref, dwq_ref, dwkT_ref, dwvT_ref, dwo_ref, dw1T_ref, dw3T_ref, dw2_ref,
            in_sems, out_sems, dx_sems, dw_sems,
            ln1_ref, k_ref, v_ref, kT_ref, v1T_ref, qf_ref, bq_ref, kmax_ref, dof_ref, df_ref, oTf_ref,
            pT_ref, sa_ref, sb_ref, dqf_ref, oTc_ref, dOT_ref, dh_ref, dqTc_ref,
            dkT_ref, dvT_ref, dwq_acc, dwo_acc, dw1_acc, dw3_acc, dw2_acc, dx_acc, ds_buf):
    in_pairs = ((x_hbm, x_ref), (wkT_hbm, wkT_ref), (wvT_hbm, wvT_ref), (wq_hbm, wq_ref),
                (wo_hbm, wo_ref), (w1T_hbm, w1T_ref), (w3T_hbm, w3T_ref), (w2_hbm, w2_ref),
                (g_hbm, g_ref))

    def in_copy(n):
        return pltpu.make_async_copy(in_pairs[n][0], in_pairs[n][1], in_sems.at[n])

    dw_pairs = ((dwq_ref, dwq_hbm), (dwo_ref, dwo_hbm), (dw1T_ref, dw1T_hbm),
                (dw3T_ref, dw3T_hbm), (dw2_ref, dw2_hbm), (dwkT_ref, dwkT_hbm),
                (dwvT_ref, dwvT_hbm))

    def dw_copy(n):
        return pltpu.make_async_copy(dw_pairs[n][0], dw_pairs[n][1], dw_sems.at[n])

    def rows_copy(src, dst, sems, blk):
        r = pl.ds(pl.multiple_of(blk * _BQ, _BQ), _BQ)
        return pltpu.make_async_copy(src.at[r, :], dst.at[r, :], sems.at[blk])

    i = pl.program_id(0)
    qbase = pl.multiple_of((i % 2) * _NCOL, _NCOL)

    @pl.when(i == 0)
    def _prologue():
        for n in range(len(in_pairs)):
            in_copy(n).start()
        for n in range(4):
            in_copy(n).wait()

        def ln_chunk(c, carry):
            r = pl.ds(pl.multiple_of(c * _BQ, _BQ), _BQ)
            xhat, _ = _ln_fwd(x_ref[r, :].astype(_f32))
            ln1 = xhat.astype(_bf16)
            ln1_ref[r, :] = ln1
            k_ref[r, :] = _mm(ln1, wkT_ref[...], _NT).astype(_bf16)
            v_ref[r, :] = _mm(ln1, wvT_ref[...], _NT).astype(_bf16)
            kT_ref[:, r] = _mm(wkT_ref[...], ln1, _NT).astype(_bf16)
            v1T_ref[0:_DH, r] = _mm(wvT_ref[...], ln1, _NT).astype(_bf16)
            return carry

        lax.fori_loop(0, _NB, ln_chunk, 0)
        row = lax.broadcasted_iota(jnp.int32, (_DH, _S), 0)
        v1T_ref[_DH:2 * _DH, :] = jnp.where(row == 0, 1.0, 0.0).astype(_bf16)
        dkT_ref[...] = jnp.zeros_like(dkT_ref)
        dvT_ref[...] = jnp.zeros_like(dvT_ref)

        def zero_a(c, carry):
            r = pl.ds(pl.multiple_of(c * 64, 64), 64)
            dwq_acc[r, :] = jnp.zeros((64, _D), _f32)
            dwo_acc[r, :] = jnp.zeros((64, _D), _f32)
            return carry

        lax.fori_loop(0, _D // 64, zero_a, 0)

        def zero_b(c, carry):
            r = pl.ds(pl.multiple_of(c * 32, 32), 32)
            dw1_acc[r, :] = jnp.zeros((32, _D), _f32)
            dw3_acc[r, :] = jnp.zeros((32, _D), _f32)
            dw2_acc[r, :] = jnp.zeros((32, _D), _f32)
            return carry

        lax.fori_loop(0, _F // 32, zero_b, 0)

        ksq = kT_ref[...].astype(_f32)
        ksq = jnp.sum(ksq * ksq, axis=0, keepdims=True)
        kmax_ref[...] = jnp.ones((1, _BQ), _f32) * jnp.sqrt(jnp.max(ksq, axis=1, keepdims=True))
        _qproj(wq_ref, ln1_ref, qf_ref, bq_ref, kmax_ref, 0, 0)

    _qproj(wq_ref, ln1_ref, qf_ref, bq_ref, kmax_ref, jnp.minimum(i + 1, _NB - 1),
           pl.multiple_of(((i + 1) % 2) * _NCOL, _NCOL))

    _attn_fwd_fast(k_ref, qf_ref, qbase, bq_ref, v1T_ref, oTf_ref, pT_ref)

    @pl.when(jnp.logical_not(jnp.min(oTf_ref[_DH:_DH + 1, :]) >= _THR))
    def _exact_forward():
        _attn_fwd(k_ref, qf_ref, qbase, v1T_ref, oTf_ref, pT_ref, sa_ref, sb_ref)

    linv = 1.0 / oTf_ref[_DH:_DH + 1, :]
    on = oTf_ref[0:_DH, :] * linv
    for h in range(_H):
        oTc_ref[h * _DH:(h + 1) * _DH, :] = on[:, h * _BQ:(h + 1) * _BQ]

    @pl.when(i == 0)
    def _wait_dense_inputs():
        for n in range(4, len(in_pairs)):
            in_copy(n).wait()

    def dense(sb, carry):
        rows = pl.ds(pl.multiple_of(i * _BQ + sb * _RB, _RB), _RB)
        lanes = pl.ds(pl.multiple_of(sb * _RB, _RB), _RB)
        xf = x_ref[rows, :].astype(_f32)
        oTc_b = oTc_ref[:, lanes].astype(_bf16)
        hres = xf + _mm(oTc_b, wo_ref[...], _TN)
        xhat2, rstd2 = _ln_fwd(hres)
        ln2 = xhat2.astype(_bf16)
        gate = _mm(ln2, w1T_ref[...], _NT)
        up = _mm(ln2, w3T_ref[...], _NT)
        sig = jax.nn.sigmoid(gate)
        silu = gate * sig
        hh = (silu * up).astype(_bf16)
        out_ref[rows, :] = (hres + jnp.dot(hh, w2_ref[...], preferred_element_type=_f32)).astype(_bf16)
        gb = g_ref[rows, :]
        d_hh = _mm(gb, w2_ref[...], _NT)
        dw2_acc[...] += _mm(hh, gb, _TN)
        d_up = (d_hh * silu).astype(_bf16)
        d_gate = (d_hh * up * (sig * (1.0 + gate * (1.0 - sig)))).astype(_bf16)
        dw1_acc[...] += _mm(d_gate, ln2, _TN)
        dw3_acc[...] += _mm(d_up, ln2, _TN)
        d_ln2 = _mm(d_gate, w1T_ref[...], _NN) + _mm(d_up, w3T_ref[...], _NN)
        dh = gb.astype(_f32) + _ln_bwd(d_ln2, xhat2, rstd2)
        dh_ref[pl.ds(pl.multiple_of(sb * _RB, _RB), _RB), :] = dh
        dhb = dh.astype(_bf16)
        dOT_ref[:, lanes] = _mm(wo_ref[...], dhb, _NT)
        dwo_acc[...] += jnp.dot(oTc_b, dhb, preferred_element_type=_f32)
        return carry

    lax.fori_loop(0, _NSB, dense, 0)
    rows_copy(out_ref, out_hbm, out_sems, i).start()

    for h in range(_H):
        li = linv[:, h * _BQ:(h + 1) * _BQ]
        dos = (dOT_ref[h * _DH:(h + 1) * _DH, :] * li).astype(_bf16)
        dof_ref[:, h * _BQ:(h + 1) * _BQ] = dos
        df_ref[:, h * _BQ:(h + 1) * _BQ] = jnp.sum(
            dos.astype(_f32) * oTc_ref[h * _DH:(h + 1) * _DH, :], axis=0, keepdims=True)

    _attn_bwd(v_ref, dof_ref, df_ref, kT_ref, qf_ref, qbase, pT_ref, dqf_ref, dkT_ref, dvT_ref, ds_buf)

    for h in range(_H):
        dqTc_ref[h * _DH:(h + 1) * _DH, :] = (dqf_ref[:, h * _BQ:(h + 1) * _BQ] * _SC).astype(_bf16)

    def qback(sb, carry):
        rows = pl.ds(pl.multiple_of(i * _BQ + sb * _RB, _RB), _RB)
        dqT_b = dqTc_ref[:, pl.ds(pl.multiple_of(sb * _RB, _RB), _RB)]
        d_ln1 = _mm(dqT_b, wq_ref[...], _T01)
        dwq_acc[...] += _mm(ln1_ref[rows, :], dqT_b, _T01)
        xhat1, rstd1 = _ln_fwd(x_ref[rows, :].astype(_f32))
        dx_acc[rows, :] = (dh_ref[pl.ds(pl.multiple_of(sb * _RB, _RB), _RB), :]
                           + _ln_bwd(d_ln1, xhat1, rstd1))
        return carry

    lax.fori_loop(0, _NSB, qback, 0)

    @pl.when(i == _NB - 1)
    def _epilogue():
        def cp_a(c, carry):
            r = pl.ds(pl.multiple_of(c * 64, 64), 64)
            dwq_ref[r, :] = dwq_acc[r, :].astype(_bf16)
            dwo_ref[r, :] = dwo_acc[r, :].astype(_bf16)
            return carry

        lax.fori_loop(0, _D // 64, cp_a, 0)

        def cp_b(c, carry):
            r = pl.ds(pl.multiple_of(c * 32, 32), 32)
            dw1T_ref[r, :] = dw1_acc[r, :].astype(_bf16)
            dw3T_ref[r, :] = dw3_acc[r, :].astype(_bf16)
            dw2_ref[r, :] = dw2_acc[r, :].astype(_bf16)
            return carry

        lax.fori_loop(0, _F // 32, cp_b, 0)
        for n in range(5):
            dw_copy(n).start()

        dkT_ref[...] = dkT_ref[...] * _LN2

        def fin(c, carry):
            awk, awv = carry
            r = pl.ds(pl.multiple_of(c * _BQ, _BQ), _BQ)
            dkb = dkT_ref[:, r].astype(_bf16)
            dvb = dvT_ref[:, r].astype(_bf16)
            ln1 = ln1_ref[r, :]
            awk = awk + _mm(dkb, ln1, _NN)
            awv = awv + _mm(dvb, ln1, _NN)
            dl = _mm(dkb, wkT_ref[...], _TN) + _mm(dvb, wvT_ref[...], _TN)
            xh, rs = _ln_fwd(x_ref[r, :].astype(_f32))
            dx_ref[r, :] = (dx_acc[r, :] + _ln_bwd(dl, xh, rs)).astype(_bf16)
            rows_copy(dx_ref, dx_hbm, dx_sems, c).start()
            return awk, awv

        z = jnp.zeros((_DH, _D), _f32)
        awk, awv = lax.fori_loop(0, _NB, fin, (z, z))
        dwkT_ref[...] = awk.astype(_bf16)
        dwvT_ref[...] = awv.astype(_bf16)
        for n in range(5, len(dw_pairs)):
            dw_copy(n).start()

        for n in range(len(dw_pairs)):
            dw_copy(n).wait()
        for blk in range(_NB):
            rows_copy(dx_ref, dx_hbm, dx_sems, blk).wait()
            rows_copy(out_ref, out_hbm, out_sems, blk).wait()


@jax.jit
def pallas_sequential_preLN__grouped_kv_mqa__glu_gated_swiglu__prompt_kernel(
    A_x: jax.Array,
    A_wq: jax.Array,
    A_wk: jax.Array,
    A_wv: jax.Array,
    A_wo: jax.Array,
    B_x: jax.Array,
    B_w1: jax.Array,
    B_w3: jax.Array,
    B_w2: jax.Array,
    grad_out: jax.Array,
):
    del B_x
    x = A_x.reshape(_S, _D)
    g = grad_out.reshape(_S, _D)
    ins = (x, A_wq, A_wk.T, A_wv.T, A_wo, B_w1.T, B_w3.T, B_w2, g)
    out_shapes = (
        jax.ShapeDtypeStruct((_S, _D), _bf16),
        jax.ShapeDtypeStruct((_S, _D), _bf16),
        jax.ShapeDtypeStruct((_D, _D), _bf16),
        jax.ShapeDtypeStruct((_DH, _D), _bf16),
        jax.ShapeDtypeStruct((_DH, _D), _bf16),
        jax.ShapeDtypeStruct((_D, _D), _bf16),
        jax.ShapeDtypeStruct((_F, _D), _bf16),
        jax.ShapeDtypeStruct((_F, _D), _bf16),
        jax.ShapeDtypeStruct((_F, _D), _bf16),
    )
    scratch = [pltpu.VMEM(a.shape, _bf16) for a in ins]
    scratch += [pltpu.VMEM(o.shape, _bf16) for o in out_shapes]
    scratch += [
        pltpu.SemaphoreType.DMA((len(ins),)),
        pltpu.SemaphoreType.DMA((_NB,)),
        pltpu.SemaphoreType.DMA((_NB,)),
        pltpu.SemaphoreType.DMA((7,)),
    ]
    scratch += [
        pltpu.VMEM((_S, _D), _bf16),
        pltpu.VMEM((_S, _DH), _bf16),
        pltpu.VMEM((_S, _DH), _bf16),
        pltpu.VMEM((_DH, _S), _bf16),
        pltpu.VMEM((2 * _DH, _S), _bf16),
        pltpu.VMEM((_DH, 2 * _NCOL), _bf16),
        pltpu.VMEM((1, 2 * _NCOL), _f32),
        pltpu.VMEM((1, _BQ), _f32),
        pltpu.VMEM((_DH, _NCOL), _bf16),
        pltpu.VMEM((1, _NCOL), _f32),
        pltpu.VMEM((2 * _DH, _NCOL), _f32),
        pltpu.VMEM((_S, _NCOL), _bf16),
        pltpu.VMEM((_S, _C), _f32),
        pltpu.VMEM((_S, _C), _f32),
        pltpu.VMEM((_DH, _NCOL), _f32),
        pltpu.VMEM((_D, _BQ), _f32),
        pltpu.VMEM((_D, _BQ), _f32),
        pltpu.VMEM((_BQ, _D), _f32),
        pltpu.VMEM((_D, _BQ), _bf16),
        pltpu.VMEM((_DH, _S), _f32),
        pltpu.VMEM((_DH, _S), _f32),
        pltpu.VMEM((_D, _D), _f32),
        pltpu.VMEM((_D, _D), _f32),
        pltpu.VMEM((_F, _D), _f32),
        pltpu.VMEM((_F, _D), _f32),
        pltpu.VMEM((_F, _D), _f32),
        pltpu.VMEM((_S, _D), _f32),
        pltpu.VMEM((_LAG + 1, _TB, _C), _bf16),
    ]
    outs = pl.pallas_call(
        _kernel,
        grid=(_NB,),
        in_specs=[pl.BlockSpec(memory_space=pl.ANY) for _ in ins],
        out_specs=[pl.BlockSpec(memory_space=pl.ANY) for _ in out_shapes],
        out_shape=out_shapes,
        scratch_shapes=scratch,
        compiler_params=pltpu.CompilerParams(
            dimension_semantics=("arbitrary",),
            vmem_limit_bytes=120 * 1024 * 1024,
        ),
    )(*ins)
    out, dx = outs[0].reshape(1, _S, _D), outs[1].reshape(1, _S, _D)
    dwq, dwkT, dwvT, dwo, dw1T, dw3T, dw2 = outs[2:]
    return (out, dx, dwq, dwkT.T, dwvT.T, dwo, dw1T.T, dw3T.T, dw2)
```
